```python
import jax
import jax.numpy as jnp

def _softmax(x, axis=-1):
    return jax.nn.softmax(x, axis=axis)
def _gelu(x):
    return jax.nn.gelu(x, approximate=True)
def _silu(x):
    return jax.nn.silu(x)
def _sigmoid(x):
    return jax.nn.sigmoid(x)
def _layernorm(x, axis=-1, eps=1e-5):
    m = jnp.mean(x, axis=axis, keepdims=True)
    v = jnp.var(x, axis=axis, keepdims=True)
    return (x - m) / jnp.sqrt(v + eps)
def _scatter_add(tgt, idx, src, axis=0):
    return tgt.at[idx].add(src)
def _segment_sum(src, seg, n):
    return jax.ops.segment_sum(src, seg, n)
class _Rng:
    def __init__(self, key):
        self._k = key
    def _next(self):
        self._k, sub = jax.random.split(self._k)
        return sub
    def normal(self, shape):
        return jax.random.normal(self._next(), shape, dtype=jnp.bfloat16)
    def randint(self, lo, hi, shape):
        return jax.random.randint(self._next(), shape, lo, hi, dtype=jnp.int32)
    def uniform(self, shape, lo=0.0, hi=1.0):
        return jax.random.uniform(self._next(), shape, jnp.bfloat16, lo, hi)
    def permutation(self, n):
        return jax.random.permutation(self._next(), n)


kernel_name = 'concat_heads__ssm_conv_h3__linear_attn_block__prompt'

def setup_inputs():
    _rng = _Rng(jax.random.key(int.from_bytes(__import__("os").urandom(4), "little")))
    _w = (lambda a: (lambda t: t.astype(jnp.bfloat16) if jnp.issubdtype(t.dtype, jnp.floating) else t)(jnp.asarray(a)))
    def _A_setup():
        B, S, D = 1, 2048, 1024
        ks = 4
        return {
            "q": _w((lambda *s: _rng.normal(s) * 0.05)(B, S, D)),
            "k": _w((lambda *s: _rng.normal(s) * 0.05)(B, S, D)),
            "v": _w((lambda *s: _rng.normal(s) * 0.05)(B, S, D)),
            "shift_k": _w((lambda *s: _rng.normal(s) * 0.05)(D, ks) * 0.5),
            "ssm_k": _w((lambda *s: _rng.normal(s) * 0.05)(D, S) * (1.0 / S ** 0.5)),
            "ssm_D": _w((lambda *s: _rng.normal(s) * 0.05)(D)),
        }
    _A_in = _A_setup()

    def _B_setup():
        B, S, D = 1, 2048, 1024
        return {
            "x": _w((lambda *s: _rng.normal(s) * 0.05)(B, S, D)),
            "wqkv": _w((lambda *s: _rng.normal(s) * 0.05)(D, 3 * D)),
            "wo": _w((lambda *s: _rng.normal(s) * 0.05)(D, D)),
        }
    _B_in = _B_setup()

    return {
        "A_q": _A_in["q"],
        "A_k": _A_in["k"],
        "A_v": _A_in["v"],
        "A_shift_k": _A_in["shift_k"],
        "A_ssm_k": _A_in["ssm_k"],
        "A_ssm_D": _A_in["ssm_D"],
        "B_x": _B_in["x"],
        "B_wqkv": _B_in["wqkv"],
        "B_wo": _B_in["wo"],
    }

def reference(A_q, A_k, A_v, A_shift_k, A_ssm_k, A_ssm_D, B_x, B_wqkv, B_wo):
    def _A_ref(q, k, v, shift_k, ssm_k, ssm_D):
        B, S, D = q.shape
        ks = shift_k.shape[-1]
        k_pad = jnp.pad(k, ((0, 0), (ks - 1, 0), (0, 0)))
        k_shift = jnp.zeros_like(k)
        for t in range(ks):
            k_shift = k_shift + k_pad[:, t:t + S, :] * shift_k[:, ks - 1 - t][None, None, :]
        kv = k_shift * v
        L = 2 * S
        kv_pad = jnp.pad(kv, ((0, 0), (0, S), (0, 0)))
        kf_pad = jnp.pad(ssm_k, ((0, 0), (0, S)))
        kv_f = (lambda x, axes=(-2,-1): jnp.fft.rfft2(x.astype(jnp.float32), axes=axes))(kv_pad[:, None, :, :], axes=(1, 2))
        kf_f = (lambda x, axes=(-2,-1): jnp.fft.rfft2(x.astype(jnp.float32), axes=axes))(kf_pad[:, None, :], axes=(1, 2))
        kf_f = (lambda x, *d: x.transpose(*d))(kf_f, 1, 2, 0)
        y_f = kv_f * kf_f[None, :, :, :]
        y = (lambda x, s, axes=(-2,-1): jnp.fft.irfft2(x, s=s, axes=axes).astype(jnp.bfloat16))(y_f, (1, L), axes=(1, 2))[:, 0, :S, :]
        y = y + kv * ssm_D[None, None, :]
        return q * y

    def _B_ref(x, wqkv, wo):
        B, S, D = x.shape
        H = 32; Dh = D // H
        qkv = (lambda x, *d: x.transpose(*d))((x @ wqkv).reshape(B, S, 3, H, Dh), 2, 0, 3, 1, 4)
        q, k, v = qkv[0], qkv[1], qkv[2]
        phi = lambda t: jnp.where(t > 0, t + 1, jnp.exp(t)) + 1e-6
        pq, pk = phi(q), phi(k)
        kv = jnp.einsum("bhsd,bhse->bhde", pk, v)
        z = jnp.einsum("bhsd->bhd", pk)
        num = jnp.einsum("bhqd,bhde->bhqe", pq, kv)
        den = jnp.einsum("bhqd,bhd->bhq", pq, z)[..., None] + 1e-6
        o = num / den
        return (lambda x, *d: x.transpose(*d))(o, 0, 2, 1, 3).reshape(B, S, D) @ wo

    a = _A_ref(A_q, A_k, A_v, A_shift_k, A_ssm_k, A_ssm_D)
    b = _B_ref(B_x, B_wqkv, B_wo)
    return jnp.concatenate([a, b], axis=-1)
```

```python
import numpy as np
import jax
import jax.numpy as jnp
import jax.experimental.pallas as pl
import jax.experimental.pallas.tpu as pltpu
import ml_dtypes

S, D, L, NC = 2048, 1024, 128, 16
T = 128
NS = D // T
f32, bf16 = jnp.float32, jnp.bfloat16


def _dft_consts():
    f = np.concatenate([np.arange(0, L, 2), np.arange(1, L, 2)])
    th = np.pi * (2 * f[:, None] + 1) * np.arange(L)[None, :] / (2 * L)
    fwd = np.concatenate([np.cos(th), -np.sin(th)], axis=0)
    inv = np.concatenate([np.cos(th).T, -np.sin(th).T], axis=1) / L
    return fwd.astype(ml_dtypes.bfloat16), inv.astype(ml_dtypes.bfloat16)


def _phi(t):
    return jnp.where(t > 0, t + 1.0, jnp.exp(t)) + 1e-6


def _kernel(q_ref, k_ref, v_ref, sk_ref, h_ref, d_ref, x_ref, wq_ref, wk_ref, wv_ref, wo_ref,
            fwd_ref, inv_ref, out_hbm,
            kf, uf, U, H, Y, QKV, R, M, oA, oB, semA, semB):
    j = pl.program_id(0)
    slot = j % 2

    kf[0:8, :] = jnp.zeros((8, T), f32)
    kf[8:8 + S, :] = k_ref[...].astype(f32)
    skT = jnp.transpose(jnp.pad(sk_ref[...].astype(f32), ((0, 0), (0, 124))))
    taps = [skT[m:m + 1, :] for m in range(4)]
    for c in range(NC):
        r0 = 8 + c * L
        ks = kf[r0:r0 + L, :] * taps[0]
        for m in range(1, 4):
            ks = ks + kf[r0 - m:r0 - m + L, :] * taps[m]
        u = ks * v_ref[c * L:(c + 1) * L, :].astype(f32)
        ub = u.astype(bf16)
        uf[c * L:(c + 1) * L, :] = ub
        U[c] = jnp.dot(fwd_ref[...], ub, preferred_element_type=f32)
        H[c] = jax.lax.dot_general(fwd_ref[...], h_ref[:, c * L:(c + 1) * L], (((1,), (1,)), ((), ())),
                                   preferred_element_type=f32)

    for ft in range(16):
        rows = slice(ft * 128, (ft + 1) * 128)
        xb = x_ref[rows, :]
        QKV[0, rows, :] = _phi(jnp.dot(xb, wq_ref[...], preferred_element_type=f32)).astype(bf16)
        QKV[1, rows, :] = _phi(jnp.dot(xb, wk_ref[...], preferred_element_type=f32)).astype(bf16)
        QKV[2, rows, :] = jnp.dot(xb, wv_ref[...], preferred_element_type=f32).astype(bf16)

        s = 1.0 if ft < 8 else -1.0
        re = slice(ft * 8, ft * 8 + 8)
        im = slice(L + ft * 8, L + ft * 8 + 8)
        gr, gi = [], []
        for dl in range(NC):
            a, b = H[dl, re, :], H[dl, im, :]
            if dl > 0:
                pa, pb = H[dl - 1, re, :], H[dl - 1, im, :]
                a, b = (a - pb, b + pa) if s > 0 else (a + pb, b - pa)
            gr.append(a); gi.append(b)
        ur = [U[c, re, :] for c in range(NC)]
        ui = [U[c, im, :] for c in range(NC)]
        for c in range(NC):
            yr = yi = None
            for dl in range(c + 1):
                a, b = ur[c - dl], ui[c - dl]
                tr = a * gr[dl] - b * gi[dl]
                ti = a * gi[dl] + b * gr[dl]
                yr = tr if yr is None else yr + tr
                yi = ti if yi is None else yi + ti
            Y[c, re, :] = yr
            Y[c, im, :] = yi

    pq, pk, vv = QKV[0], QKV[1], QKV[2]
    ri = jax.lax.broadcasted_iota(jnp.int32, (T, T), 0) // 32
    ci = jax.lax.broadcasted_iota(jnp.int32, (T, T), 1) // 32
    bd = ri == ci
    kv = jax.lax.dot_general(pk, vv, (((0,), (0,)), ((), ())), preferred_element_type=f32)
    kv = jnp.where(bd, kv, 0.0).astype(bf16)
    z = jnp.sum(pk.astype(f32), axis=0, keepdims=True)
    zc = jnp.transpose(jnp.broadcast_to(z, (T, T)))
    zbd = jnp.where(bd, zc, 0.0).astype(bf16)
    den = jnp.dot(pq, zbd, preferred_element_type=f32) + 1e-6
    col = pl.ds(pl.multiple_of(j * T, T), T)
    R[:, col] = (pq.astype(f32) / den).astype(bf16)
    M[col, :] = jnp.dot(kv, wo_ref[...], preferred_element_type=f32).astype(bf16)

    @pl.when(j >= 2)
    def _():
        pltpu.make_async_copy(oA.at[slot], out_hbm.at[:, col], semA.at[slot]).wait()
    dv = d_ref[...].astype(f32)
    for c in range(NC):
        r = slice(c * L, (c + 1) * L)
        y = jnp.dot(inv_ref[...], Y[c].astype(bf16), preferred_element_type=f32)
        y = y + uf[r, :].astype(f32) * dv
        oA[slot, r, :] = (q_ref[r, :].astype(f32) * y).astype(bf16)
    pltpu.make_async_copy(oA.at[slot], out_hbm.at[:, col], semA.at[slot]).start()

    @pl.when(j == NS - 1)
    def _():
        RB = 256
        for b in range(S // RB):
            r = slice(b * RB, (b + 1) * RB)
            oB[r, :] = jnp.dot(R[r, :], M[...], preferred_element_type=f32).astype(bf16)
            pltpu.make_async_copy(oB.at[r, :], out_hbm.at[r, D:2 * D], semB.at[b]).start()
        for b in range(S // RB):
            r = slice(b * RB, (b + 1) * RB)
            pltpu.make_async_copy(oB.at[r, :], out_hbm.at[r, D:2 * D], semB.at[b]).wait()
        for sl in range(2):
            pltpu.make_async_copy(oA.at[sl], out_hbm.at[:, 0:T], semA.at[sl]).wait()


@jax.jit
def pallas_concat_heads__ssm_conv_h3__linear_attn_block__prompt_kernel(
    A_q, A_k, A_v, A_shift_k, A_ssm_k, A_ssm_D, B_x, B_wqkv, B_wo,
):
    fwd, inv = _dft_consts()
    tile = pl.BlockSpec((S, T), lambda j: (0, j))
    in_specs = [
        tile, tile, tile,
        pl.BlockSpec((T, 4), lambda j: (j, 0)),
        pl.BlockSpec((T, S), lambda j: (j, 0)),
        pl.BlockSpec((1, T), lambda j: (0, j)),
        pl.BlockSpec((S, D), lambda j: (0, 0)),
        pl.BlockSpec((D, T), lambda j: (0, j)),
        pl.BlockSpec((D, T), lambda j: (0, NS + j)),
        pl.BlockSpec((D, T), lambda j: (0, 2 * NS + j)),
        pl.BlockSpec((T, D), lambda j: (j, 0)),
        pl.BlockSpec((2 * L, L), lambda j: (0, 0)),
        pl.BlockSpec((L, 2 * L), lambda j: (0, 0)),
    ]
    scratch = [
        pltpu.VMEM((S + 8, T), f32),
        pltpu.VMEM((S, T), bf16),
        pltpu.VMEM((NC, 2 * L, T), f32),
        pltpu.VMEM((NC, 2 * L, T), f32),
        pltpu.VMEM((NC, 2 * L, T), f32),
        pltpu.VMEM((3, S, T), bf16),
        pltpu.VMEM((S, D), bf16),
        pltpu.VMEM((D, D), bf16),
        pltpu.VMEM((2, S, T), bf16),
        pltpu.VMEM((S, D), bf16),
        pltpu.SemaphoreType.DMA((2,)),
        pltpu.SemaphoreType.DMA((8,)),
    ]
    out = pl.pallas_call(
        _kernel,
        grid=(NS,),
        in_specs=in_specs,
        out_specs=pl.BlockSpec(memory_space=pl.ANY),
        out_shape=jax.ShapeDtypeStruct((S, 2 * D), bf16),
        scratch_shapes=scratch,
        compiler_params=pltpu.CompilerParams(
            dimension_semantics=("arbitrary",), vmem_limit_bytes=100 * 2**20),
    )(A_q[0], A_k[0], A_v[0], A_shift_k, A_ssm_k, A_ssm_D.reshape(1, D), B_x[0],
      B_wqkv, B_wqkv, B_wqkv, B_wo, fwd, inv)
    return out[None]
```

```python
import numpy as np
import jax
import jax.numpy as jnp
import jax.experimental.pallas as pl
import jax.experimental.pallas.tpu as pltpu
import ml_dtypes

S, D, L, NC = 2048, 1024, 128, 16
T = 128
NS = D // T
f32, bf16 = jnp.float32, jnp.bfloat16


def _dft_consts():
    f = np.concatenate([np.arange(0, L, 2), np.arange(1, L, 2)])
    th = np.pi * (2 * f[:, None] + 1) * np.arange(L)[None, :] / (2 * L)
    fwd = np.concatenate([np.cos(th), -np.sin(th)], axis=0)
    inv = np.concatenate([np.cos(th).T, -np.sin(th).T], axis=1) / L
    return fwd.astype(ml_dtypes.bfloat16), inv.astype(ml_dtypes.bfloat16)


SCHED = [1, 2, 2, 3, 4, 5, 6, 7, 8, 9, 10, 11, 13, 15, 16, 17, 18]
LAG = 1


def _rcp(d):
    r = pl.reciprocal(d, approx=True)
    return r * (2.0 - d * r)


def _phi(t):
    return jnp.where(t > 0, t + 1.0, jnp.exp(t)) + 1e-6


def _kernel(q_hbm, k_hbm, v_hbm, sk_hbm, h_hbm, d_hbm, x_hbm, w_hbm, wo_hbm, fwd_hbm, inv_hbm, out_hbm,
            q2, k2, v2, h2, wq2, wk2, wv2, wo2, sk_all, d_all, x_ref, fwd_ref, inv_ref,
            kf, uf, U, H, G, Y, QKV, R, M, oA, oB, semA, semB, semI, semX, semC):
    def tiles(j, sl):
        col = pl.ds(pl.multiple_of(j * T, T), T)
        wc = lambda o: pl.ds(pl.multiple_of(o + j * T, T), T)
        cp = pltpu.make_async_copy
        return [cp(w_hbm.at[:, wc(D)], wk2.at[sl], semI.at[sl, 0]),
                cp(w_hbm.at[:, wc(2 * D)], wv2.at[sl], semI.at[sl, 1]),
                cp(k_hbm.at[:, col], k2.at[sl], semI.at[sl, 2]),
                cp(v_hbm.at[:, col], v2.at[sl], semI.at[sl, 3]),
                cp(h_hbm.at[col, :], h2.at[sl], semI.at[sl, 4]),
                cp(q_hbm.at[:, col], q2.at[sl], semI.at[sl, 5]),
                cp(w_hbm.at[:, wc(0)], wq2.at[sl], semI.at[sl, 6]),
                cp(wo_hbm.at[col, :], wo2.at[sl], semI.at[sl, 7])]

    xcp = [pltpu.make_async_copy(x_hbm.at[b * 256:(b + 1) * 256, :], x_ref.at[b * 256:(b + 1) * 256, :], semX.at[b])
           for b in range(8)]
    ccp = [pltpu.make_async_copy(s_, d_, semC.at[i]) for i, (s_, d_) in enumerate(
        [(sk_hbm, sk_all), (d_hbm, d_all), (fwd_hbm, fwd_ref), (inv_hbm, inv_ref)])]
    t0 = tiles(0, 0)
    first = t0[:5] + ccp + xcp[:2]
    for c_ in first:
        c_.start()
    for c_ in xcp[2:] + t0[5:]:
        c_.start()
    for c_ in ccp + xcp:
        c_.wait()

    def step(j, is_first):
        slot = j % 2
        if is_first:
            pre = {2 * b: [xcp[b]] for b in range(2, 8)}
            pre[16] = [t0[6], t0[7]]
            late = t0[5]
        else:
            pre, late = {}, None
            for c_ in tiles(j, slot):
                c_.wait()

        @pl.when(j + 1 < NS)
        def _():
            for c_ in tiles(j + 1, 1 - slot):
                c_.start()
        _step(j, slot, pre, late, q2.at[slot], k2.at[slot], v2.at[slot], sk_all, h2.at[slot], d_all, x_ref,
              wq2.at[slot], wk2.at[slot], wv2.at[slot], wo2.at[slot], fwd_ref, inv_ref, out_hbm,
              kf, uf, U, H, G, Y, QKV, R, M, oA, semA)

    pass

    def body(j, c):
        step(j, False)
        return c
    jax.lax.fori_loop(0, NS, body, 0)
    RB = 256
    for b in range(S // RB):
        r = slice(b * RB, (b + 1) * RB)
        oB[r, :] = jnp.dot(R[r, :], M[...], preferred_element_type=f32).astype(bf16)
        pltpu.make_async_copy(oB.at[r, :], out_hbm.at[r, D:2 * D], semB.at[b]).start()
    for b in range(S // RB):
        r = slice(b * RB, (b + 1) * RB)
        pltpu.make_async_copy(oB.at[r, :], out_hbm.at[r, D:2 * D], semB.at[b]).wait()
    for sl in range(2):
        pltpu.make_async_copy(oA.at[sl], out_hbm.at[:, 0:T], semA.at[sl]).wait()


def _step(j, slot, pre, late, q_ref, k_ref, v_ref, sk_all, h_ref, d_all, x_ref, wq_ref, wk_ref, wv_ref, wo_ref,
          fwd_ref, inv_ref, out_hbm, kf, uf, U, H, G, Y, QKV, R, M, oA, semA):
    col = pl.ds(pl.multiple_of(j * T, T), T)
    kf[0:8, :] = jnp.zeros((8, T), f32)
    kf[8:8 + S, :] = k_ref[...].astype(f32)
    skT = jnp.transpose(jnp.pad(sk_all[col, :].astype(f32), ((0, 0), (0, 124))))
    taps = [skT[m:m + 1, :] for m in range(4)]
    ri = jax.lax.broadcasted_iota(jnp.int32, (T, T), 0) // 32
    ci = jax.lax.broadcasted_iota(jnp.int32, (T, T), 1) // 32
    bd = ri == ci
    dv = d_all[:, col].astype(f32)

    @pl.when(j >= 2)
    def _():
        pltpu.make_async_copy(oA.at[slot], out_hbm.at[:, col], semA.at[slot]).wait()

    def a_fwd(c):
        r0 = 8 + c * L
        ks = kf[r0:r0 + L, :] * taps[0]
        for m in range(1, 4):
            ks = ks + kf[r0 - m:r0 - m + L, :] * taps[m]
        ub = (ks * v_ref[c * L:(c + 1) * L, :].astype(f32)).astype(bf16)
        uf[c * L:(c + 1) * L, :] = ub
        U[c] = jnp.dot(fwd_ref[...], ub, preferred_element_type=f32)
        hh = jax.lax.dot_general(fwd_ref[...], h_ref[:, c * L:(c + 1) * L], (((1,), (1,)), ((), ())),
                                 preferred_element_type=f32)
        H[c] = hh
        if c == 0:
            G[c] = hh
        else:
            p = H[c - 1]
            h2 = L // 2
            G[c, 0:h2] = hh[0:h2] - p[L:L + h2]
            G[c, h2:L] = hh[h2:L] + p[L + h2:2 * L]
            G[c, L:L + h2] = hh[L:L + h2] + p[0:h2]
            G[c, L + h2:2 * L] = hh[L + h2:2 * L] - p[h2:L]

    def a_conv(c):
        for ft in range(16):
            re = slice(ft * 8, ft * 8 + 8)
            im = slice(L + ft * 8, L + ft * 8 + 8)
            yr = yi = None
            for dl in range(c + 1):
                a, b = U[c - dl, re, :], U[c - dl, im, :]
                gr, gi = G[dl, re, :], G[dl, im, :]
                tr = a * gr - b * gi
                ti = a * gi + b * gr
                yr = tr if yr is None else yr + tr
                yi = ti if yi is None else yi + ti
            Y[c, re, :] = yr
            Y[c, im, :] = yi

    def a_inv(c):
        if c == 0 and late is not None:
            late.wait()
        r = slice(c * L, (c + 1) * L)
        y = jnp.dot(inv_ref[...], Y[c].astype(bf16), preferred_element_type=f32)
        y = y + uf[r, :].astype(f32) * dv
        oA[slot, r, :] = (q_ref[r, :].astype(f32) * y).astype(bf16)

    st = {}
    RB = 256

    def b_unit(n):
        for c_ in pre.get(n, []):
            c_.wait()
        if n < 16:
            r = slice((n // 2) * RB, (n // 2 + 1) * RB)
            if n % 2 == 0:
                QKV[1, r, :] = _phi(jnp.dot(x_ref[r, :], wk_ref[...], preferred_element_type=f32)).astype(bf16)
            else:
                QKV[2, r, :] = jnp.dot(x_ref[r, :], wv_ref[...], preferred_element_type=f32).astype(bf16)
        if n == 16:
            pk, vv = QKV[1], QKV[2]
            kv = jax.lax.dot_general(pk, vv, (((0,), (0,)), ((), ())), preferred_element_type=f32)
            kv = jnp.where(bd, kv, 0.0).astype(bf16)
            z = jnp.sum(pk.astype(f32), axis=0, keepdims=True)
            zc = jnp.transpose(jnp.broadcast_to(z, (T, T)))
            st["zbd"] = jnp.where(bd, zc, 0.0).astype(bf16)
            M[col, :] = jnp.dot(kv, wo_ref[...], preferred_element_type=f32).astype(bf16)
        if n >= 16:
            r = slice((n - 16) * RB, (n - 15) * RB)
            pq = _phi(jnp.dot(x_ref[r, :], wq_ref[...], preferred_element_type=f32)).astype(bf16)
            den = jnp.dot(pq, st["zbd"], preferred_element_type=f32) + 1e-6
            R[r, col] = (pq.astype(f32) * _rcp(den)).astype(bf16)

    nb = 0
    for c in range(NC + LAG):
        if c < NC:
            a_fwd(c)
        tgt = SCHED[c] if c < len(SCHED) else 24
        while nb < tgt:
            b_unit(nb); nb += 1
        if c >= LAG:
            a_inv(c - LAG)
        if c < NC:
            a_conv(c)
    pltpu.make_async_copy(oA.at[slot], out_hbm.at[:, col], semA.at[slot]).start()


@jax.jit
def pallas_concat_heads__ssm_conv_h3__linear_attn_block__prompt_kernel(
    A_q, A_k, A_v, A_shift_k, A_ssm_k, A_ssm_D, B_x, B_wqkv, B_wo,
):
    fwd, inv = _dft_consts()
    in_specs = [pl.BlockSpec(memory_space=pl.ANY)] * 11
    scratch = [
        pltpu.VMEM((2, S, T), bf16), pltpu.VMEM((2, S, T), bf16), pltpu.VMEM((2, S, T), bf16),
        pltpu.VMEM((2, T, S), bf16),
        pltpu.VMEM((2, D, T), bf16), pltpu.VMEM((2, D, T), bf16), pltpu.VMEM((2, D, T), bf16),
        pltpu.VMEM((2, T, D), bf16),
        pltpu.VMEM((D, 4), bf16), pltpu.VMEM((1, D), bf16), pltpu.VMEM((S, D), bf16),
        pltpu.VMEM((2 * L, L), bf16), pltpu.VMEM((L, 2 * L), bf16),
        pltpu.VMEM((S + 8, T), f32),
        pltpu.VMEM((S, T), bf16),
        pltpu.VMEM((NC, 2 * L, T), f32),
        pltpu.VMEM((NC, 2 * L, T), f32),
        pltpu.VMEM((NC, 2 * L, T), f32),
        pltpu.VMEM((NC, 2 * L, T), f32),
        pltpu.VMEM((3, S, T), bf16),
        pltpu.VMEM((S, D), bf16),
        pltpu.VMEM((D, D), bf16),
        pltpu.VMEM((2, S, T), bf16),
        pltpu.VMEM((S, D), bf16),
        pltpu.SemaphoreType.DMA((2,)),
        pltpu.SemaphoreType.DMA((8,)),
        pltpu.SemaphoreType.DMA((2, 8)),
        pltpu.SemaphoreType.DMA((8,)),
        pltpu.SemaphoreType.DMA((4,)),
    ]
    out = pl.pallas_call(
        _kernel,
        in_specs=in_specs,
        out_specs=pl.BlockSpec(memory_space=pl.ANY),
        out_shape=jax.ShapeDtypeStruct((S, 2 * D), bf16),
        scratch_shapes=scratch,
        compiler_params=pltpu.CompilerParams(
            vmem_limit_bytes=100 * 2**20),
    )(A_q[0], A_k[0], A_v[0], A_shift_k, A_ssm_k, A_ssm_D.reshape(1, D), B_x[0],
      B_wqkv, B_wo, fwd, inv)
    return out[None]
```

```python
import numpy as np
import jax
import jax.numpy as jnp
import jax.experimental.pallas as pl
import jax.experimental.pallas.tpu as pltpu
import ml_dtypes

S, D, L, NC = 2048, 1024, 128, 16
T = 128
NS = D // T
f32, bf16 = jnp.float32, jnp.bfloat16


def _dft_consts():
    f = np.concatenate([np.arange(0, L, 2), np.arange(1, L, 2)])
    th = np.pi * (2 * f[:, None] + 1) * np.arange(L)[None, :] / (2 * L)
    fwd = np.concatenate([np.cos(th), -np.sin(th)], axis=0)
    inv = np.concatenate([np.cos(th).T, -np.sin(th).T], axis=1) / L
    return fwd.astype(ml_dtypes.bfloat16), inv.astype(ml_dtypes.bfloat16)


SCHED = [1,2,3,4,5,6,8,9,11,12,14,16,17,19,21,23,24]
LAG = 1


def _rcp(d):
    r = pl.reciprocal(d, approx=True)
    return r * (2.0 - d * r)


def _phi(t):
    return jnp.where(t > 0, t + 1.0, jnp.exp(t)) + 1e-6


def _kernel(q_hbm, k_hbm, v_hbm, sk_hbm, h_hbm, d_hbm, x_hbm, w_hbm, wo_hbm, fwd_hbm, inv_hbm, out_hbm,
            q2, k2, v2, h2, wq2, wk2, wv2, wo2, sk_all, d_all, x_ref, fwd_ref, inv_ref,
            kf, uf, U, H, G, Y, QKV, R, M, oA, oB, semA, semB, semI, semX, semC):
    def tiles(j, sl):
        col = pl.ds(pl.multiple_of(j * T, T), T)
        wc = lambda o: pl.ds(pl.multiple_of(o + j * T, T), T)
        cp = pltpu.make_async_copy
        return [cp(w_hbm.at[:, wc(D)], wk2.at[sl], semI.at[sl, 0]),
                cp(w_hbm.at[:, wc(2 * D)], wv2.at[sl], semI.at[sl, 1]),
                cp(k_hbm.at[:, col], k2.at[sl], semI.at[sl, 2]),
                cp(v_hbm.at[:, col], v2.at[sl], semI.at[sl, 3]),
                cp(h_hbm.at[col, :], h2.at[sl], semI.at[sl, 4]),
                cp(q_hbm.at[:, col], q2.at[sl], semI.at[sl, 5]),
                cp(w_hbm.at[:, wc(0)], wq2.at[sl], semI.at[sl, 6]),
                cp(wo_hbm.at[col, :], wo2.at[sl], semI.at[sl, 7])]

    xcp = [pltpu.make_async_copy(x_hbm.at[b * 256:(b + 1) * 256, :], x_ref.at[b * 256:(b + 1) * 256, :], semX.at[b])
           for b in range(8)]
    ccp = [pltpu.make_async_copy(s_, d_, semC.at[i]) for i, (s_, d_) in enumerate(
        [(sk_hbm, sk_all), (d_hbm, d_all), (fwd_hbm, fwd_ref), (inv_hbm, inv_ref)])]
    t0 = tiles(0, 0)
    first = t0[:5] + ccp + xcp[:2]
    for c_ in first:
        c_.start()
    for c_ in xcp[2:] + t0[5:]:
        c_.start()
    for c_ in ccp + xcp:
        c_.wait()

    def step(j, is_first):
        slot = j % 2
        if is_first:
            pre = {2 * b: [xcp[b]] for b in range(2, 8)}
            pre[16] = [t0[6], t0[7]]
            late = t0[5]
        else:
            pre, late = {}, None
            for c_ in tiles(j, slot):
                c_.wait()

        @pl.when(j + 1 < NS)
        def _():
            for c_ in tiles(j + 1, 1 - slot):
                c_.start()
        _step(j, slot, pre, late, q2.at[slot], k2.at[slot], v2.at[slot], sk_all, h2.at[slot], d_all, x_ref,
              wq2.at[slot], wk2.at[slot], wv2.at[slot], wo2.at[slot], fwd_ref, inv_ref, out_hbm,
              kf, uf, U, H, G, Y, QKV, R, M, oA, semA)

    pass

    def body(j, c):
        step(j, False)
        return c
    jax.lax.fori_loop(0, NS, body, 0)
    RB = 256
    for b in range(S // RB):
        r = slice(b * RB, (b + 1) * RB)
        oB[r, :] = jnp.dot(R[r, :], M[...], preferred_element_type=f32).astype(bf16)
        pltpu.make_async_copy(oB.at[r, :], out_hbm.at[r, D:2 * D], semB.at[b]).start()
    for b in range(S // RB):
        r = slice(b * RB, (b + 1) * RB)
        pltpu.make_async_copy(oB.at[r, :], out_hbm.at[r, D:2 * D], semB.at[b]).wait()
    for sl in range(2):
        pltpu.make_async_copy(oA.at[sl], out_hbm.at[:, 0:T], semA.at[sl]).wait()


def _step(j, slot, pre, late, q_ref, k_ref, v_ref, sk_all, h_ref, d_all, x_ref, wq_ref, wk_ref, wv_ref, wo_ref,
          fwd_ref, inv_ref, out_hbm, kf, uf, U, H, G, Y, QKV, R, M, oA, semA):
    col = pl.ds(pl.multiple_of(j * T, T), T)
    kf[0:8, :] = jnp.zeros((8, T), f32)
    kf[8:8 + S, :] = k_ref[...].astype(f32)
    skT = jnp.transpose(jnp.pad(sk_all[col, :].astype(f32), ((0, 0), (0, 124))))
    taps = [skT[m:m + 1, :] for m in range(4)]
    ri = jax.lax.broadcasted_iota(jnp.int32, (T, T), 0) // 32
    ci = jax.lax.broadcasted_iota(jnp.int32, (T, T), 1) // 32
    bd = ri == ci
    dv = d_all[:, col].astype(f32)

    @pl.when(j >= 2)
    def _():
        pltpu.make_async_copy(oA.at[slot], out_hbm.at[:, col], semA.at[slot]).wait()

    def a_fwd(c):
        r0 = 8 + c * L
        ks = kf[r0:r0 + L, :] * taps[0]
        for m in range(1, 4):
            ks = ks + kf[r0 - m:r0 - m + L, :] * taps[m]
        ub = (ks * v_ref[c * L:(c + 1) * L, :].astype(f32)).astype(bf16)
        uf[c * L:(c + 1) * L, :] = ub
        U[c] = jnp.dot(fwd_ref[...], ub, preferred_element_type=f32)
        hh = jax.lax.dot_general(fwd_ref[...], h_ref[:, c * L:(c + 1) * L], (((1,), (1,)), ((), ())),
                                 preferred_element_type=f32)
        H[c] = hh
        if c == 0:
            G[c] = hh
        else:
            p = H[c - 1]
            h2 = L // 2
            G[c, 0:h2] = hh[0:h2] - p[L:L + h2]
            G[c, h2:L] = hh[h2:L] + p[L + h2:2 * L]
            G[c, L:L + h2] = hh[L:L + h2] + p[0:h2]
            G[c, L + h2:2 * L] = hh[L + h2:2 * L] - p[h2:L]

    def a_conv(c):
        for ft in range(16):
            re = slice(ft * 8, ft * 8 + 8)
            im = slice(L + ft * 8, L + ft * 8 + 8)
            yr = yi = None
            for dl in range(c + 1):
                a, b = U[c - dl, re, :], U[c - dl, im, :]
                gr, gi = G[dl, re, :], G[dl, im, :]
                tr = a * gr - b * gi
                ti = a * gi + b * gr
                yr = tr if yr is None else yr + tr
                yi = ti if yi is None else yi + ti
            Y[c, re, :] = yr
            Y[c, im, :] = yi

    def a_inv(c):
        if c == 0 and late is not None:
            late.wait()
        r = slice(c * L, (c + 1) * L)
        y = jnp.dot(inv_ref[...], Y[c].astype(bf16), preferred_element_type=f32)
        y = y + uf[r, :].astype(f32) * dv
        oA[slot, r, :] = (q_ref[r, :].astype(f32) * y).astype(bf16)

    st = {}
    RB = 256

    def b_unit(n):
        for c_ in pre.get(n, []):
            c_.wait()
        if n < 24:
            r = slice((n % 8) * RB, (n % 8 + 1) * RB)
            p = jnp.dot(x_ref[r, :], (wq_ref, wk_ref, wv_ref)[n // 8][...], preferred_element_type=f32)
            QKV[n // 8, r, :] = (_phi(p) if n < 16 else p).astype(bf16)
        elif n == 24:
            pk, vv = QKV[1], QKV[2]
            kv = jax.lax.dot_general(pk, vv, (((0,), (0,)), ((), ())), preferred_element_type=f32)
            kv = jnp.where(bd, kv, 0.0).astype(bf16)
            M[col, :] = jnp.dot(kv, wo_ref[...], preferred_element_type=f32).astype(bf16)
        if n == 16:
            z = jnp.sum(QKV[1].astype(f32), axis=0, keepdims=True)
            zc = jnp.transpose(jnp.broadcast_to(z, (T, T)))
            st["zbd"] = jnp.where(bd, zc, 0.0).astype(bf16)
        if 16 <= n < 24:
            r = slice((n - 16) * RB, (n - 15) * RB)
            pq = QKV[0, r, :]
            den = jnp.dot(pq, st["zbd"], preferred_element_type=f32) + 1e-6
            R[r, col] = (pq.astype(f32) * _rcp(den)).astype(bf16)

    nb = 0
    for c in range(NC + LAG):
        if c < NC:
            a_fwd(c)
        tgt = SCHED[c] if c < len(SCHED) else 24
        while nb < tgt:
            b_unit(nb); nb += 1
        if c >= LAG:
            a_inv(c - LAG)
        if c < NC:
            a_conv(c)
    pltpu.make_async_copy(oA.at[slot], out_hbm.at[:, col], semA.at[slot]).start()
    while nb < 25:
        b_unit(nb); nb += 1


@jax.jit
def pallas_concat_heads__ssm_conv_h3__linear_attn_block__prompt_kernel(
    A_q, A_k, A_v, A_shift_k, A_ssm_k, A_ssm_D, B_x, B_wqkv, B_wo,
):
    fwd, inv = _dft_consts()
    in_specs = [pl.BlockSpec(memory_space=pl.ANY)] * 11
    scratch = [
        pltpu.VMEM((2, S, T), bf16), pltpu.VMEM((2, S, T), bf16), pltpu.VMEM((2, S, T), bf16),
        pltpu.VMEM((2, T, S), bf16),
        pltpu.VMEM((2, D, T), bf16), pltpu.VMEM((2, D, T), bf16), pltpu.VMEM((2, D, T), bf16),
        pltpu.VMEM((2, T, D), bf16),
        pltpu.VMEM((D, 4), bf16), pltpu.VMEM((1, D), bf16), pltpu.VMEM((S, D), bf16),
        pltpu.VMEM((2 * L, L), bf16), pltpu.VMEM((L, 2 * L), bf16),
        pltpu.VMEM((S + 8, T), f32),
        pltpu.VMEM((S, T), bf16),
        pltpu.VMEM((NC, 2 * L, T), f32),
        pltpu.VMEM((NC, 2 * L, T), f32),
        pltpu.VMEM((NC, 2 * L, T), f32),
        pltpu.VMEM((NC, 2 * L, T), f32),
        pltpu.VMEM((3, S, T), bf16),
        pltpu.VMEM((S, D), bf16),
        pltpu.VMEM((D, D), bf16),
        pltpu.VMEM((2, S, T), bf16),
        pltpu.VMEM((S, D), bf16),
        pltpu.SemaphoreType.DMA((2,)),
        pltpu.SemaphoreType.DMA((8,)),
        pltpu.SemaphoreType.DMA((2, 8)),
        pltpu.SemaphoreType.DMA((8,)),
        pltpu.SemaphoreType.DMA((4,)),
    ]
    out = pl.pallas_call(
        _kernel,
        in_specs=in_specs,
        out_specs=pl.BlockSpec(memory_space=pl.ANY),
        out_shape=jax.ShapeDtypeStruct((S, 2 * D), bf16),
        scratch_shapes=scratch,
        compiler_params=pltpu.CompilerParams(
            vmem_limit_bytes=100 * 2**20),
    )(A_q[0], A_k[0], A_v[0], A_shift_k, A_ssm_k, A_ssm_D.reshape(1, D), B_x[0],
      B_wqkv, B_wo, fwd, inv)
    return out[None]
```

```python
import numpy as np
import jax
import jax.numpy as jnp
import jax.experimental.pallas as pl
import jax.experimental.pallas.tpu as pltpu
import ml_dtypes

S, D, L, NC = 2048, 1024, 128, 16
T = 128
NS = D // T
f32, bf16 = jnp.float32, jnp.bfloat16


def _dft_consts():
    f = np.concatenate([np.arange(0, L, 2), np.arange(1, L, 2)])
    th = np.pi * (2 * f[:, None] + 1) * np.arange(L)[None, :] / (2 * L)
    fwd = np.concatenate([np.cos(th), -np.sin(th)], axis=0)
    inv = np.concatenate([np.cos(th).T, -np.sin(th).T], axis=1) / L
    return fwd.astype(ml_dtypes.bfloat16), inv.astype(ml_dtypes.bfloat16)


SCHED = [1,2,3,4,5,6,8,9,11,12,14,16,17,19,21,23,24]
LAG = 1


def _rcp(d):
    r = pl.reciprocal(d, approx=True)
    return r * (2.0 - d * r)


def _phi(t):
    return jnp.where(t > 0, t + 1.0, jnp.exp(t)) + 1e-6


def _kernel(q_hbm, k_hbm, v_hbm, sk_hbm, h_hbm, d_hbm, x_hbm, w_hbm, wo_hbm, fwd_hbm, inv_hbm, out_hbm,
            q2, k2, v2, h2, wq2, wk2, wv2, wo2, sk_all, d_all, x_ref, fwd_ref, inv_ref,
            kf, uf, U, H, G, Y, QKV, R, M, oA, oB, semA, semB, semI, semX, semC):
    def tiles(j, sl):
        col = pl.ds(pl.multiple_of(j * T, T), T)
        wc = lambda o: pl.ds(pl.multiple_of(o + j * T, T), T)
        cp = pltpu.make_async_copy
        return [cp(w_hbm.at[:, wc(D)], wk2.at[sl], semI.at[sl, 0]),
                cp(w_hbm.at[:, wc(2 * D)], wv2.at[sl], semI.at[sl, 1]),
                cp(k_hbm.at[:, col], k2.at[sl], semI.at[sl, 2]),
                cp(v_hbm.at[:, col], v2.at[sl], semI.at[sl, 3]),
                cp(h_hbm.at[col, :], h2.at[sl], semI.at[sl, 4]),
                cp(q_hbm.at[:, col], q2.at[sl], semI.at[sl, 5]),
                cp(w_hbm.at[:, wc(0)], wq2.at[sl], semI.at[sl, 6]),
                cp(wo_hbm.at[col, :], wo2.at[sl], semI.at[sl, 7])]

    xcp = [pltpu.make_async_copy(x_hbm.at[b * 256:(b + 1) * 256, :], x_ref.at[b * 256:(b + 1) * 256, :], semX.at[b])
           for b in range(8)]
    ccp = [pltpu.make_async_copy(s_, d_, semC.at[i]) for i, (s_, d_) in enumerate(
        [(sk_hbm, sk_all), (d_hbm, d_all), (fwd_hbm, fwd_ref), (inv_hbm, inv_ref)])]
    t0 = tiles(0, 0)
    first = t0[:5] + ccp + xcp[:2]
    for c_ in first:
        c_.start()
    for c_ in xcp[2:] + t0[5:]:
        c_.start()
    for c_ in ccp + xcp:
        c_.wait()

    def step(j, is_first):
        slot = j % 2
        if is_first:
            pre = {2 * b: [xcp[b]] for b in range(2, 8)}
            pre[16] = [t0[6], t0[7]]
            late = t0[5]
        else:
            pre, late = {}, None
            for c_ in tiles(j, slot):
                c_.wait()

        @pl.when(j + 1 < NS)
        def _():
            for c_ in tiles(j + 1, 1 - slot):
                c_.start()
        _step(j, slot, pre, late, q2.at[slot], k2.at[slot], v2.at[slot], sk_all, h2.at[slot], d_all, x_ref,
              wq2.at[slot], wk2.at[slot], wv2.at[slot], wo2.at[slot], fwd_ref, inv_ref, out_hbm,
              kf, uf, U, H, G, Y, QKV, R, M, oA, semA)

    pass

    def body(j, c):
        step(j, False)
        return c
    jax.lax.fori_loop(0, NS, body, 0)
    RB = 256
    for b in range(S // RB):
        r = slice(b * RB, (b + 1) * RB)
        oB[r, :] = jnp.dot(R[r, :], M[...], preferred_element_type=f32).astype(bf16)
        pltpu.make_async_copy(oB.at[r, :], out_hbm.at[r, D:2 * D], semB.at[b]).start()
    for b in range(S // RB):
        r = slice(b * RB, (b + 1) * RB)
        pltpu.make_async_copy(oB.at[r, :], out_hbm.at[r, D:2 * D], semB.at[b]).wait()
    for sl in range(2):
        pltpu.make_async_copy(oA.at[sl], out_hbm.at[:, 0:T], semA.at[sl]).wait()


def _step(j, slot, pre, late, q_ref, k_ref, v_ref, sk_all, h_ref, d_all, x_ref, wq_ref, wk_ref, wv_ref, wo_ref,
          fwd_ref, inv_ref, out_hbm, kf, uf, U, H, G, Y, QKV, R, M, oA, semA):
    col = pl.ds(pl.multiple_of(j * T, T), T)
    kf[0:8, :] = jnp.zeros((8, T), f32)
    kf[8:8 + S, :] = k_ref[...].astype(f32)
    skT = jnp.transpose(jnp.pad(sk_all[col, :].astype(f32), ((0, 0), (0, 124))))
    taps = [skT[m:m + 1, :] for m in range(4)]
    ri = jax.lax.broadcasted_iota(jnp.int32, (T, T), 0) // 32
    ci = jax.lax.broadcasted_iota(jnp.int32, (T, T), 1) // 32
    bd = ri == ci
    dv = d_all[:, col].astype(f32)

    @pl.when(j >= 2)
    def _():
        pltpu.make_async_copy(oA.at[slot], out_hbm.at[:, col], semA.at[slot]).wait()

    def a_fwd(c):
        r0 = 8 + c * L
        ks = kf[r0:r0 + L, :] * taps[0]
        for m in range(1, 4):
            ks = ks + kf[r0 - m:r0 - m + L, :] * taps[m]
        ub = (ks * v_ref[c * L:(c + 1) * L, :].astype(f32)).astype(bf16)
        uf[c * L:(c + 1) * L, :] = ub
        uu = jnp.dot(fwd_ref[...], ub, preferred_element_type=f32)
        U[c, 0:2 * L] = uu
        U[c, 2 * L:3 * L] = uu[0:L] + uu[L:2 * L]
        hh = jax.lax.dot_general(fwd_ref[...], h_ref[:, c * L:(c + 1) * L], (((1,), (1,)), ((), ())),
                                 preferred_element_type=f32)
        H[c] = hh
        gr, gi = hh[0:L], hh[L:2 * L]
        if c > 0:
            p = H[c - 1]
            h2 = L // 2
            gr = jnp.concatenate([gr[0:h2] - p[L:L + h2], gr[h2:L] + p[L + h2:2 * L]], axis=0)
            gi = jnp.concatenate([gi[0:h2] + p[0:h2], gi[h2:L] - p[h2:L]], axis=0)
        G[c, 0:L] = gr
        G[c, L:2 * L] = gi - gr
        G[c, 2 * L:3 * L] = gi + gr

    def a_conv(c):
        for ft in range(16):
            re = slice(ft * 8, ft * 8 + 8)
            im = slice(L + ft * 8, L + ft * 8 + 8)
            sm = slice(2 * L + ft * 8, 2 * L + ft * 8 + 8)
            k1 = k2 = k3 = None
            for dl in range(c + 1):
                t1 = G[dl, re, :] * U[c - dl, sm, :]
                t2 = G[dl, im, :] * U[c - dl, re, :]
                t3 = G[dl, sm, :] * U[c - dl, im, :]
                k1, k2, k3 = (t1, t2, t3) if k1 is None else (k1 + t1, k2 + t2, k3 + t3)
            Y[c, re, :] = k1 - k3
            Y[c, im, :] = k1 + k2

    def a_inv(c):
        if c == 0 and late is not None:
            late.wait()
        r = slice(c * L, (c + 1) * L)
        y = jnp.dot(inv_ref[...], Y[c].astype(bf16), preferred_element_type=f32)
        y = y + uf[r, :].astype(f32) * dv
        oA[slot, r, :] = (q_ref[r, :].astype(f32) * y).astype(bf16)

    st = {}
    RB = 256

    def b_unit(n):
        for c_ in pre.get(n, []):
            c_.wait()
        if n < 24:
            r = slice((n % 8) * RB, (n % 8 + 1) * RB)
            p = jnp.dot(x_ref[r, :], (wq_ref, wk_ref, wv_ref)[n // 8][...], preferred_element_type=f32)
            QKV[n // 8, r, :] = (_phi(p) if n < 16 else p).astype(bf16)
        elif n == 24:
            pk, vv = QKV[1], QKV[2]
            kv = jax.lax.dot_general(pk, vv, (((0,), (0,)), ((), ())), preferred_element_type=f32)
            kv = jnp.where(bd, kv, 0.0).astype(bf16)
            M[col, :] = jnp.dot(kv, wo_ref[...], preferred_element_type=f32).astype(bf16)
        if n == 16:
            z = jnp.sum(QKV[1].astype(f32), axis=0, keepdims=True)
            zc = jnp.transpose(jnp.broadcast_to(z, (T, T)))
            st["zbd"] = jnp.where(bd, zc, 0.0).astype(bf16)
        if 16 <= n < 24:
            r = slice((n - 16) * RB, (n - 15) * RB)
            pq = QKV[0, r, :]
            den = jnp.dot(pq, st["zbd"], preferred_element_type=f32) + 1e-6
            R[r, col] = (pq.astype(f32) * _rcp(den)).astype(bf16)

    nb = 0
    for c in range(NC + LAG):
        if c < NC:
            a_fwd(c)
        tgt = SCHED[c] if c < len(SCHED) else 24
        while nb < tgt:
            b_unit(nb); nb += 1
        if c >= LAG:
            a_inv(c - LAG)
        if c < NC:
            a_conv(c)
    pltpu.make_async_copy(oA.at[slot], out_hbm.at[:, col], semA.at[slot]).start()
    while nb < 25:
        b_unit(nb); nb += 1


@jax.jit
def pallas_concat_heads__ssm_conv_h3__linear_attn_block__prompt_kernel(
    A_q, A_k, A_v, A_shift_k, A_ssm_k, A_ssm_D, B_x, B_wqkv, B_wo,
):
    fwd, inv = _dft_consts()
    in_specs = [pl.BlockSpec(memory_space=pl.ANY)] * 11
    scratch = [
        pltpu.VMEM((2, S, T), bf16), pltpu.VMEM((2, S, T), bf16), pltpu.VMEM((2, S, T), bf16),
        pltpu.VMEM((2, T, S), bf16),
        pltpu.VMEM((2, D, T), bf16), pltpu.VMEM((2, D, T), bf16), pltpu.VMEM((2, D, T), bf16),
        pltpu.VMEM((2, T, D), bf16),
        pltpu.VMEM((D, 4), bf16), pltpu.VMEM((1, D), bf16), pltpu.VMEM((S, D), bf16),
        pltpu.VMEM((2 * L, L), bf16), pltpu.VMEM((L, 2 * L), bf16),
        pltpu.VMEM((S + 8, T), f32),
        pltpu.VMEM((S, T), bf16),
        pltpu.VMEM((NC, 3 * L, T), f32),
        pltpu.VMEM((NC, 2 * L, T), f32),
        pltpu.VMEM((NC, 3 * L, T), f32),
        pltpu.VMEM((NC, 2 * L, T), f32),
        pltpu.VMEM((3, S, T), bf16),
        pltpu.VMEM((S, D), bf16),
        pltpu.VMEM((D, D), bf16),
        pltpu.VMEM((2, S, T), bf16),
        pltpu.VMEM((S, D), bf16),
        pltpu.SemaphoreType.DMA((2,)),
        pltpu.SemaphoreType.DMA((8,)),
        pltpu.SemaphoreType.DMA((2, 8)),
        pltpu.SemaphoreType.DMA((8,)),
        pltpu.SemaphoreType.DMA((4,)),
    ]
    out = pl.pallas_call(
        _kernel,
        in_specs=in_specs,
        out_specs=pl.BlockSpec(memory_space=pl.ANY),
        out_shape=jax.ShapeDtypeStruct((S, 2 * D), bf16),
        scratch_shapes=scratch,
        compiler_params=pltpu.CompilerParams(
            vmem_limit_bytes=100 * 2**20),
    )(A_q[0], A_k[0], A_v[0], A_shift_k, A_ssm_k, A_ssm_D.reshape(1, D), B_x[0],
      B_wqkv, B_wo, fwd, inv)
    return out[None]
```
